```python
import os as _os
_os.environ.setdefault("JAX_PLATFORMS", "cpu")
import jax
import jax.numpy as jnp

def _softmax(x, axis=-1):
    return jax.nn.softmax(x, axis=axis)
def _gelu(x):
    return jax.nn.gelu(x, approximate=True)
def _silu(x):
    return jax.nn.silu(x)
def _sigmoid(x):
    return jax.nn.sigmoid(x)
def _layernorm(x, axis=-1, eps=1e-5):
    m = jnp.mean(x, axis=axis, keepdims=True)
    v = jnp.var(x, axis=axis, keepdims=True)
    return (x - m) / jnp.sqrt(v + eps)
def _scatter_add(tgt, idx, src, axis=0):
    return tgt.at[idx].add(src)
def _segment_sum(src, seg, n):
    return jax.ops.segment_sum(src, seg, n)
class _Rng:
    def __init__(self, key):
        self._k = key
    def _next(self):
        self._k, sub = jax.random.split(self._k)
        return sub
    def normal(self, shape):
        return jax.random.normal(self._next(), shape, dtype=jnp.bfloat16)
    def randint(self, lo, hi, shape):
        return jax.random.randint(self._next(), shape, lo, hi, dtype=jnp.int32)
    def uniform(self, shape, lo=0.0, hi=1.0):
        return jax.random.uniform(self._next(), shape, jnp.bfloat16, lo, hi)
    def permutation(self, n):
        return jax.random.permutation(self._next(), n)


kernel_name = 'standalone__dense_activation_silu__prompt'

def setup_inputs():
    _rng = _Rng(jax.random.key(int.from_bytes(__import__("os").urandom(4), "little")))
    _w = (lambda a: (lambda t: t.astype(jnp.bfloat16) if jnp.issubdtype(t.dtype, jnp.floating) else t)(jnp.asarray(a)))
    B, S, D, F = 1, 2048, 448, 1792
    return {
        "x": _w((lambda *s: _rng.normal(s) * 0.05)(B, S, D)),
        "w1": _w((lambda *s: _rng.normal(s) * 0.05)(D, F) * (D ** -0.5)),
        "w2": _w((lambda *s: _rng.normal(s) * 0.05)(F, D) * (F ** -0.5)),
    }

def reference(x, w1, w2):
    h = jnp.einsum("bsd,df->bsf", x, w1)
    h = _silu(h)
    out = jnp.einsum("bsf,fd->bsd", h, w2)
    return out
```

```python
import jax
import jax.numpy as jnp
import jax.experimental.pallas as pl
import jax.experimental.pallas.tpu as pltpu

_TILE = 512
_W1_CUT = 512


def _silu(h):
    return h / (1.0 + jnp.exp(-h))


def _ffn_kernel(xT_hbm, w1_hbm, w2T_hbm, oT_hbm, x_v, w1_v, w1T_v, w2_v, o_v, a_v, sem):
    D, S = xT_hbm.shape
    F = w1_hbm.shape[1]
    bf16, f32 = jnp.bfloat16, jnp.float32

    def copy(src, dst, c0, c1, k):
        cols = pl.ds(c0, c1 - c0)
        return pltpu.make_async_copy(src.at[:, cols], dst.at[:, cols], sem.at[k])

    cx0 = copy(xT_hbm, x_v, 0, _TILE, 0)
    c1 = [copy(w1_hbm, w1_v, 0, _W1_CUT, 1), copy(w1_hbm, w1_v, _W1_CUT, F, 2)]
    c2 = copy(w2T_hbm, w2_v, 0, F, 3)
    cxr = copy(xT_hbm, x_v, _TILE, S, 4)
    for c in [cx0, *c1, c2, cxr]:
        c.start()

    cx0.wait()
    for c, (f0, f1) in zip(c1, [(0, _W1_CUT), (_W1_CUT, F)]):
        c.wait()
        wt = w1_v[:, f0:f1].T
        w1T_v[f0:f1, :] = wt
        hT = jnp.dot(wt, x_v[:, 0:_TILE], preferred_element_type=f32)
        a_v[f0:f1, :] = _silu(hT).astype(bf16)
    c2.wait()
    cxr.wait()
    o_v[:, 0:_TILE] = jnp.dot(w2_v[...], a_v[...], preferred_element_type=f32).astype(bf16)
    co0 = copy(o_v, oT_hbm, 0, S - _TILE, 5)
    co1 = copy(o_v, oT_hbm, S - _TILE, S, 6)
    for s0 in range(_TILE, S, _TILE):
        if s0 == S - _TILE:
            co0.start()
        hT = jnp.dot(w1T_v[...], x_v[:, s0:s0 + _TILE], preferred_element_type=f32)
        a = _silu(hT).astype(bf16)
        o_v[:, s0:s0 + _TILE] = jnp.dot(w2_v[...], a, preferred_element_type=f32).astype(bf16)
    co1.start()
    co0.wait()
    co1.wait()


@jax.jit
def pallas_standalone__dense_activation_silu__prompt_kernel(
    x: jax.Array,
    w1: jax.Array,
    w2: jax.Array,
):
    B, S, D = x.shape
    F = w1.shape[1]
    bf16 = jnp.bfloat16
    xT = x.reshape(B * S, D).T
    w2T = w2.T
    oT = pl.pallas_call(
        _ffn_kernel,
        in_specs=[pl.BlockSpec(memory_space=pl.ANY)] * 3,
        out_specs=pl.BlockSpec(memory_space=pl.ANY),
        out_shape=jax.ShapeDtypeStruct((D, B * S), x.dtype),
        scratch_shapes=[
            pltpu.VMEM((D, B * S), bf16),
            pltpu.VMEM((D, F), bf16),
            pltpu.VMEM((F, D), bf16),
            pltpu.VMEM((D, F), bf16),
            pltpu.VMEM((D, B * S), bf16),
            pltpu.VMEM((F, _TILE), bf16),
            pltpu.SemaphoreType.DMA((7,)),
        ],
        compiler_params=pltpu.CompilerParams(vmem_limit_bytes=100 * 1024 * 1024),
    )(xT, w1, w2T)
    return oT.T.reshape(B, S, D)
```

```python
import numpy as np

import jax
import jax.numpy as jnp
from jax import lax
import jax.experimental.pallas as pl
import jax.experimental.pallas.tpu as pltpu

_U = 128
_NEG_LOG2E = -1.4426950408889634
_F32_MAX = float(np.finfo(np.float32).max)

_STAGES = ((3, 2), (4, 5), (5, 14))
_PROGRAM = (
    ("o", 0, 4), ("h", 5, 9), ("o", 4, 8), ("h", 9, 13), ("o", 8, 12),
    ("store", 0, 12), ("h", 13, 16), ("o", 12, 15),
    ("store", 12, 15), ("o", 15, 16), ("store", 15, 16),
)


def _silu(h):
    d = jnp.minimum(1.0 + jnp.exp2(h * _NEG_LOG2E), _F32_MAX)
    r = pltpu.reciprocal(d, approx=True)
    return h * (r * (2.0 - d * r))


def _ffn_kernel(xT_hbm, w1_hbm, w2T_hbm, oT_hbm,
                xT_v, w1_v, w2T_v, x_v, hid_v, oT_v, sem):
    bf16, f32 = jnp.bfloat16, jnp.float32
    n_s = xT_hbm.shape[1] // _U
    n_f = w1_hbm.shape[1] // _U
    n_stages = len(_STAGES)

    def blocks(b0, b1):
        return pl.ds(b0 * _U, (b1 - b0) * _U)

    def copy(src, dst, b0, b1, k):
        cols = blocks(b0, b1)
        return pltpu.make_async_copy(src.at[:, cols], dst.at[:, cols], sem.at[k])

    loads = []
    ps = pf = 0
    for k, (s, f) in enumerate(_STAGES):
        loads.append([copy(xT_hbm, xT_v, ps, s, k if k else n_stages + 1),
                      copy(w1_hbm, w1_v, pf, f, k)])
        ps, pf = s, f
    loads.append([copy(w2T_hbm, w2T_v, 0, n_f, n_stages),
                  copy(xT_hbm, xT_v, ps, n_s, n_stages)])
    for group in loads:
        for c in group:
            c.start()

    def transpose_x(s0, s1):
        x_v[blocks(s0, s1), :] = xT_v[:, blocks(s0, s1)].T

    def hidden(s0, s1, f0, f1):
        h = jnp.dot(x_v[blocks(s0, s1), :], w1_v[:, blocks(f0, f1)],
                    preferred_element_type=f32)
        return _silu(h).astype(bf16)

    ps = pf = 0
    for k, (s, f) in enumerate(_STAGES):
        load_x, load_w1 = loads[k]
        load_x.wait()
        if k == 0:
            transpose_x(ps, s)
        load_w1.wait()
        if k > 0:
            hid_v[blocks(0, ps), blocks(pf, f)] = hidden(0, ps, pf, f)
            transpose_x(ps, s)
        hid_v[blocks(ps, s), blocks(0, f)] = hidden(ps, s, 0, f)
        ps, pf = s, f
    for c in loads[n_stages]:
        c.wait()

    hid = {}
    stores = []
    for op, s0, s1 in _PROGRAM:
        if op == "h":
            transpose_x(s0, s1)
            a = hidden(s0, s1, 0, n_f)
            for b in range(s0, s1):
                hid[b] = a[(b - s0) * _U:(b - s0 + 1) * _U]
        elif op == "o":
            a = jnp.concatenate(
                [hid[b] if b in hid else hid_v[blocks(b, b + 1), :]
                 for b in range(s0, s1)], axis=0)
            oT = lax.dot_general(w2T_v[...], a, (((1,), (1,)), ((), ())),
                                 preferred_element_type=f32)
            oT_v[:, blocks(s0, s1)] = oT.astype(oT_v.dtype)
        else:
            stores.append(copy(oT_v, oT_hbm, s0, s1, 0))
            stores[-1].start()
    for c in stores:
        c.wait()


@jax.jit
def pallas_standalone__dense_activation_silu__prompt_kernel(
    x: jax.Array,
    w1: jax.Array,
    w2: jax.Array,
):
    B, S, D = x.shape
    F = w1.shape[1]
    T = B * S
    assert T == _PROGRAM[-1][2] * _U and F == _STAGES[-1][1] * _U
    oT = pl.pallas_call(
        _ffn_kernel,
        in_specs=[pl.BlockSpec(memory_space=pl.ANY)] * 3,
        out_specs=pl.BlockSpec(memory_space=pl.ANY),
        out_shape=jax.ShapeDtypeStruct((D, T), x.dtype),
        scratch_shapes=[
            pltpu.VMEM((D, T), x.dtype),
            pltpu.VMEM((D, F), w1.dtype),
            pltpu.VMEM((D, F), w2.dtype),
            pltpu.VMEM((T, D), x.dtype),
            pltpu.VMEM((_STAGES[-1][0] * _U, F), jnp.bfloat16),
            pltpu.VMEM((D, T), x.dtype),
            pltpu.SemaphoreType.DMA((len(_STAGES) + 2,)),
        ],
        compiler_params=pltpu.CompilerParams(
            vmem_limit_bytes=100 * 1024 * 1024,
            flags={"XLA_TPU_EVENLY_DISTRIBUTE_CRITICAL_NODES": True},
        ),
    )(x.reshape(T, D).T, w1, w2.T)
    return oT.T.reshape(B, S, D)
```

```python
import numpy as np

import jax
import jax.numpy as jnp
from jax import lax
import jax.experimental.pallas as pl
import jax.experimental.pallas.tpu as pltpu

_U = 128
_NEG_LOG2E = -1.4426950408889634
_F32_MAX = float(np.finfo(np.float32).max)

_STAGES = ((2, 3), (4, 5), (8, 9))
_PROGRAM = (
    ("finish", 0, 4), ("out", 0, 4),
    ("finish", 4, 8), ("out", 4, 8),
    ("hidden", 8, 12), ("out", 8, 12), ("store", 0, 12),
    ("hidden", 12, 16), ("out", 12, 15), ("store", 12, 15),
    ("out", 15, 16), ("store", 15, 16),
)


def _silu(h):
    d = jnp.minimum(1.0 + jnp.exp2(h * _NEG_LOG2E), _F32_MAX)
    r = pltpu.reciprocal(d, approx=True)
    return h * (r * (2.0 - d * r))


def _ffn_kernel(xT_hbm, w1_hbm, w2T_hbm, oT_hbm,
                xT_v, w1_v, x_v, w2T_v, oT_v, hid_v, sem):
    bf16, f32 = jnp.bfloat16, jnp.float32
    n_s = xT_hbm.shape[1] // _U
    n_f = w1_hbm.shape[1] // _U
    s_early, f_early = _STAGES[-1]

    def blocks(b0, b1):
        return pl.ds(b0 * _U, (b1 - b0) * _U)

    def copy(src, dst, b0, b1, k):
        cols = blocks(b0, b1)
        return pltpu.make_async_copy(src.at[:, cols], dst.at[:, cols], sem.at[k])

    s, f = _STAGES[0]
    loads = [[copy(xT_hbm, xT_v, 0, s, 0)], [copy(w1_hbm, w1_v, 0, f, 1)]]
    for (ps, pf), (s, f) in zip(_STAGES, _STAGES[1:]):
        k = len(loads) % 2
        loads.append([copy(xT_hbm, xT_v, ps, s, k), copy(w1_hbm, w1_v, pf, f, k)])
    k = len(loads) % 2
    loads.append([copy(w1_hbm, w1_v, f_early, n_f, k),
                  copy(w2T_hbm, w2T_v, 0, n_f, k),
                  copy(xT_hbm, xT_v, s_early, n_s, k)])

    def start(g):
        if g < len(loads):
            for c in loads[g]:
                c.start()

    def wait(g):
        for c in loads[g]:
            c.wait()
        start(g + 2)

    def transpose_x(s0, s1):
        x_v[blocks(s0, s1), :] = xT_v[:, blocks(s0, s1)].T

    def hidden(s0, s1, f0, f1):
        h = jnp.dot(x_v[blocks(s0, s1), :], w1_v[:, blocks(f0, f1)],
                    preferred_element_type=f32)
        return _silu(h).astype(bf16)

    start(0)
    start(1)
    s, f = _STAGES[0]
    wait(0)
    transpose_x(0, s)
    wait(1)
    hid_v[blocks(0, s), blocks(0, f)] = hidden(0, s, 0, f)
    for g, ((ps, pf), (s, f)) in enumerate(zip(_STAGES, _STAGES[1:]), start=2):
        wait(g)
        hid_v[blocks(0, ps), blocks(pf, f)] = hidden(0, ps, pf, f)
        transpose_x(ps, s)
        hid_v[blocks(ps, s), blocks(0, f)] = hidden(ps, s, 0, f)
    wait(len(loads) - 1)

    early, late, stores = set(range(s_early)), {}, []

    def hidden_block(b):
        if b in early:
            return jnp.concatenate([hid_v[blocks(b, b + 1), :], late[b]], axis=1)
        return late[b]

    for op, s0, s1 in _PROGRAM:
        if op == "out":
            a = jnp.concatenate([hidden_block(b) for b in range(s0, s1)], axis=0)
            oT = lax.dot_general(w2T_v[...], a, (((1,), (1,)), ((), ())),
                                 preferred_element_type=f32)
            oT_v[:, blocks(s0, s1)] = oT.astype(oT_v.dtype)
        elif op == "store":
            stores.append(copy(oT_v, oT_hbm, s0, s1, 0))
            stores[-1].start()
        else:
            if op == "hidden":
                transpose_x(s0, s1)
            a = hidden(s0, s1, f_early if op == "finish" else 0, n_f)
            for b in range(s0, s1):
                late[b] = a[(b - s0) * _U:(b - s0 + 1) * _U]
    for c in stores:
        c.wait()


@jax.jit
def pallas_standalone__dense_activation_silu__prompt_kernel(
    x: jax.Array,
    w1: jax.Array,
    w2: jax.Array,
):
    B, S, D = x.shape
    F = w1.shape[1]
    T = B * S
    s_early, f_early = _STAGES[-1]
    assert T == _PROGRAM[-1][2] * _U and F % _U == 0 and F > f_early * _U
    oT = pl.pallas_call(
        _ffn_kernel,
        in_specs=[pl.BlockSpec(memory_space=pl.ANY)] * 3,
        out_specs=pl.BlockSpec(memory_space=pl.ANY),
        out_shape=jax.ShapeDtypeStruct((D, T), x.dtype),
        scratch_shapes=[
            pltpu.VMEM((D, T), x.dtype),
            pltpu.VMEM((D, F), w1.dtype),
            pltpu.VMEM((T, D), x.dtype),
            pltpu.VMEM((D, F), w2.dtype),
            pltpu.VMEM((D, T), x.dtype),
            pltpu.VMEM((s_early * _U, f_early * _U), jnp.bfloat16),
            pltpu.SemaphoreType.DMA((2,)),
        ],
        compiler_params=pltpu.CompilerParams(
            vmem_limit_bytes=100 * 1024 * 1024,
            flags={"XLA_TPU_EVENLY_DISTRIBUTE_CRITICAL_NODES": True},
        ),
    )(x.reshape(T, D).T, w1, w2.T)
    return oT.T.reshape(B, S, D)
```
